```python
import jax
import jax.numpy as jnp

def _softmax(x, axis=-1):
    return jax.nn.softmax(x, axis=axis)

def _gelu(x):
    return jax.nn.gelu(x, approximate=True)

def _silu(x):
    return jax.nn.silu(x)

def _sigmoid(x):
    return jax.nn.sigmoid(x)

def _layernorm(x, axis=-1, eps=1e-05):
    m = jnp.mean(x, axis=axis, keepdims=True)
    v = jnp.var(x, axis=axis, keepdims=True)
    return (x - m) / jnp.sqrt(v + eps)

def _scatter_add(tgt, idx, src, axis=0):
    return tgt.at[idx].add(src)

def _segment_sum(src, seg, n):
    return jax.ops.segment_sum(src, seg, n)

class _Rng:

    def __init__(self, key):
        self._k = key

    def _next(self):
        self._k, sub = jax.random.split(self._k)
        return sub

    def normal(self, shape):
        return jax.random.normal(self._next(), shape, dtype=jnp.bfloat16)

    def randint(self, lo, hi, shape):
        return jax.random.randint(self._next(), shape, lo, hi, dtype=jnp.int32)

    def uniform(self, shape, lo=0.0, hi=1.0):
        return jax.random.uniform(self._next(), shape, jnp.bfloat16, lo, hi)

    def permutation(self, n):
        return jax.random.permutation(self._next(), n)
kernel_name = 'adaLN_cond__sliding_block_cached__geglu_ffn__decode'

def setup_inputs():
    _rng = _Rng(jax.random.key(int.from_bytes(__import__("os").urandom(4), "little")))
    _w = lambda a: (lambda t: t.astype(jnp.bfloat16) if jnp.issubdtype(t.dtype, jnp.floating) else t)(jnp.asarray(a))

    def _A_setup():
        B, Sq, D = (1, 1, 640)
        Hq, Hkv, Sk, Dh = (32, 32, 32768, 192)
        assert Hq % Hkv == 0, (Hq, Hkv)
        return {'x': _w((lambda *s: _rng.normal(s) * 0.05)(B, Sq, D)), 'k_cache': _w((lambda *s: _rng.normal(s) * 0.05)(B, Hkv, Sk, Dh)), 'v_cache': _w((lambda *s: _rng.normal(s) * 0.05)(B, Hkv, Sk, Dh)), 'wq': _w((lambda *s: _rng.normal(s) * 0.05)(D, Hq * Dh) * D ** (-0.5)), 'wo': _w((lambda *s: _rng.normal(s) * 0.05)(Hq * Dh, D) * (Hq * Dh) ** (-0.5))}
    _A_in = _A_setup()

    def _B_setup():
        B, S, D, F = (1, 1, 640, 1536)
        return {'x': _w((lambda *s: _rng.normal(s) * 0.05)(B, S, D)), 'w_gate': _w((lambda *s: _rng.normal(s) * 0.05)(D, F)), 'w_up': _w((lambda *s: _rng.normal(s) * 0.05)(D, F)), 'w_down': _w((lambda *s: _rng.normal(s) * 0.05)(F, D))}
    _B_in = _B_setup()
    return {'A_x': _A_in['x'], 'A_k_cache': _A_in['k_cache'], 'A_v_cache': _A_in['v_cache'], 'A_wq': _A_in['wq'], 'A_wo': _A_in['wo'], 'B_x': _B_in['x'], 'B_w_gate': _B_in['w_gate'], 'B_w_up': _B_in['w_up'], 'B_w_down': _B_in['w_down'], 'c': _w((lambda *s: _rng.normal(s) * 0.05)(1, 640)), 'w_mod': _w((lambda *s: _rng.normal(s) * 0.05)(640, 6 * 640) * 640 ** (-0.5))}

def reference(A_x, A_k_cache, A_v_cache, A_wq, A_wo, B_x, B_w_gate, B_w_up, B_w_down, c, w_mod):

    def _A_ref(x, k_cache, v_cache, wq, wo):
        B, Sq, D = x.shape
        Hq, Dh = (32, 192)
        Hkv, Sk = (k_cache.shape[1], k_cache.shape[2])
        W = min(4096, max(256, Sk // 4))
        rep = Hq // Hkv
        q = (lambda x, *d: x.transpose(*d))((x @ wq).reshape(B, Sq, Hq, Dh), 0, 2, 1, 3)
        k = jnp.repeat(k_cache[:, :, Sk - W:, :], rep, axis=1)
        v = jnp.repeat(v_cache[:, :, Sk - W:, :], rep, axis=1)
        scores = jnp.einsum('bhqd,bhkd->bhqk', q, k) * Dh ** (-0.5)
        p = _softmax(scores, axis=-1)
        o = jnp.einsum('bhqk,bhkd->bhqd', p, v)
        return (lambda x, *d: x.transpose(*d))(o, 0, 2, 1, 3).reshape(B, Sq, Hq * Dh) @ wo

    def _B_ref(x, w_gate, w_up, w_down):
        return _gelu(x @ w_gate) * (x @ w_up) @ w_down
    x = A_x
    mod = (_silu(c) @ w_mod).reshape(c.shape[0], 6, 1, -1)
    sa, ca, ga, sb, cb, gb = (mod[:, 0].copy(), mod[:, 1].copy(), mod[:, 2].copy(), mod[:, 3].copy(), mod[:, 4].copy(), mod[:, 5].copy())
    h = _layernorm(x, axis=-1) * (1 + ca) + sa
    x = x + ga * _A_ref(h, A_k_cache, A_v_cache, A_wq, A_wo)
    h = _layernorm(x, axis=-1) * (1 + cb) + sb
    x = x + gb * _B_ref(h, B_w_gate, B_w_up, B_w_down)
    return x
```

```python
import functools

import jax
import jax.numpy as jnp
import jax.experimental.pallas as pl
import jax.experimental.pallas.tpu as pltpu

F32 = jnp.float32
BF16 = jnp.bfloat16

M = 8
NSLOT = 4
WQ_CHUNKS = 5
FC = 256


def _layernorm(x, eps=1e-5):
    m = jnp.mean(x, axis=-1, keepdims=True)
    d = x - m
    v = jnp.mean(d * d, axis=-1, keepdims=True)
    return d * jax.lax.rsqrt(v + eps)


def _gelu_tanh(x):
    c0 = 0.7978845608028654
    return 0.5 * x * (1.0 + jnp.tanh(c0 * (x + 0.044715 * (x * x * x))))


def _mm(a, b):
    return jnp.dot(a, b, preferred_element_type=F32)


def _kernel(x_hbm, kT_hbm, vT_hbm, wq_hbm, wo_hbm, wg_hbm, wu_hbm, wd_hbm, c_hbm, wm_hbm,
            o_ref,
            x_v, c_v, wm_v, wq_v, wo_v, wg_v, wu_v, wd_v, k_v, v_v, q_s, sems,
            *, H, DH, S, W, D, F):
    NP = H // 2
    NF = F // FC
    QR = D // WQ_CHUNKS

    S_X, S_C, S_WMA, S_WMB = 0, 1, 2, 3
    S_WQ = 4
    S_K = S_WQ + WQ_CHUNKS
    S_V = S_K + NSLOT
    S_WO = S_V + NSLOT
    S_G = S_WO + NP
    S_U = S_G + NF
    S_D = S_U + NF

    cp_x = pltpu.make_async_copy(x_hbm, x_v, sems.at[S_X])
    cp_c = pltpu.make_async_copy(c_hbm, c_v, sems.at[S_C])
    cp_wma = pltpu.make_async_copy(wm_hbm.at[:, pl.ds(0, 2 * D)], wm_v.at[:, pl.ds(0, 2 * D)], sems.at[S_WMA])
    cp_wmb = pltpu.make_async_copy(wm_hbm.at[:, pl.ds(2 * D, 4 * D)], wm_v.at[:, pl.ds(2 * D, 4 * D)], sems.at[S_WMB])

    def cp_wq(i):
        return pltpu.make_async_copy(wq_hbm.at[pl.ds(i * QR, QR), :], wq_v.at[pl.ds(i * QR, QR), :], sems.at[S_WQ + i])

    def cp_k(h):
        s = h % NSLOT
        return pltpu.make_async_copy(kT_hbm.at[h, :, pl.ds(S - W, W)], k_v.at[s], sems.at[S_K + s])

    def cp_v(h):
        s = h % NSLOT
        return pltpu.make_async_copy(vT_hbm.at[h, :, pl.ds(S - W, W)], v_v.at[s], sems.at[S_V + s])

    def cp_wo(j):
        r = pl.multiple_of(j * 2 * DH, 2 * DH) if not isinstance(j, int) else j * 2 * DH
        return pltpu.make_async_copy(wo_hbm.at[pl.ds(r, 2 * DH), :], wo_v.at[j], sems.at[S_WO + j])

    def cp_g(i):
        return pltpu.make_async_copy(wg_hbm.at[:, pl.ds(i * FC, FC)], wg_v.at[i], sems.at[S_G + i])

    def cp_u(i):
        return pltpu.make_async_copy(wu_hbm.at[:, pl.ds(i * FC, FC)], wu_v.at[i], sems.at[S_U + i])

    def cp_d(i):
        return pltpu.make_async_copy(wd_hbm.at[pl.ds(i * FC, FC), :], wd_v.at[i], sems.at[S_D + i])

    cp_c.start()
    cp_x.start()
    cp_wma.start()
    for i in range(WQ_CHUNKS):
        cp_wq(i).start()
    cp_k(0).start()
    cp_v(0).start()
    cp_k(1).start()

    cp_c.wait()
    cp_x.wait()
    cf = c_v[...].astype(F32)
    sc = cf * jax.nn.sigmoid(cf)
    sc8 = jnp.broadcast_to(sc, (M, D)).astype(BF16)
    xf = x_v[...].astype(F32)
    ln1 = _layernorm(xf)
    cp_wma.wait()
    mod_a = _mm(sc8, wm_v[:, 0:2 * D])
    h = ln1 * (1.0 + mod_a[:, D:2 * D]) + mod_a[:, 0:D]
    hb = h.astype(BF16)

    q = None
    for i in range(WQ_CHUNKS):
        cp_wq(i).wait()
        part = _mm(hb[:, i * QR:(i + 1) * QR], wq_v[i * QR:(i + 1) * QR, :])
        q = part if q is None else q + part
    q_s[...] = q.astype(BF16)

    scale = DH ** -0.5

    def head(hh, qh, first):
        s_ = hh % NSLOT
        cp_k(hh).wait()
        if first:
            cp_v(hh + 1).start()
            cp_wo(hh // 2).start()
        else:
            @pl.when(hh + 1 < H)
            def _():
                cp_v(hh + 1).start()
        sc_ = _mm(qh, k_v[s_]) * scale
        mx = jnp.max(sc_, axis=-1, keepdims=True)
        e = jnp.exp(sc_ - mx)
        l = jnp.sum(e, axis=-1, keepdims=True)
        cp_v(hh).wait()

        @pl.when(hh + 2 < H)
        def _():
            cp_k(hh + 2).start()
        o = jax.lax.dot_general(e.astype(BF16), v_v[s_], (((1,), (1,)), ((), ())),
                                preferred_element_type=F32)
        return o / l

    def pair(j, acc):
        qp = q_s[:, pl.ds(pl.multiple_of(j * 2 * DH, 2 * DH), 2 * DH)]
        oa = head(2 * j, qp[:, 0:DH], True)
        ob = head(2 * j + 1, qp[:, DH:2 * DH], False)
        op = jnp.concatenate([oa, ob], axis=-1).astype(BF16)
        cp_wo(j).wait()
        return acc + _mm(op, wo_v[j])

    acc = jax.lax.fori_loop(0, NP - 1, pair, jnp.zeros((M, D), F32))

    j = NP - 1
    qp = q_s[:, j * 2 * DH:(j + 1) * 2 * DH]
    cp_k(H - 2).wait()
    cp_v(H - 1).start()
    cp_wo(j).start()
    sa_ = _mm(qp[:, 0:DH], k_v[(H - 2) % NSLOT]) * scale
    e = jnp.exp(sa_ - jnp.max(sa_, axis=-1, keepdims=True))
    l = jnp.sum(e, axis=-1, keepdims=True)
    cp_v(H - 2).wait()
    cp_wmb.start()
    oa = jax.lax.dot_general(e.astype(BF16), v_v[(H - 2) % NSLOT], (((1,), (1,)), ((), ())),
                             preferred_element_type=F32) / l
    cp_k(H - 1).wait()
    cp_g(0).start()
    cp_u(0).start()
    cp_d(0).start()
    sb_ = _mm(qp[:, DH:2 * DH], k_v[(H - 1) % NSLOT]) * scale
    e = jnp.exp(sb_ - jnp.max(sb_, axis=-1, keepdims=True))
    l = jnp.sum(e, axis=-1, keepdims=True)
    cp_v(H - 1).wait()
    for i in range(1, NF):
        cp_g(i).start()
        cp_u(i).start()
        cp_d(i).start()
    ob = jax.lax.dot_general(e.astype(BF16), v_v[(H - 1) % NSLOT], (((1,), (1,)), ((), ())),
                             preferred_element_type=F32) / l
    op = jnp.concatenate([oa, ob], axis=-1).astype(BF16)
    cp_wo(j).wait()
    attn = acc + _mm(op, wo_v[j])

    cp_wmb.wait()
    mod_b = _mm(sc8, wm_v[:, 2 * D:6 * D])
    ga = mod_b[:, 0:D]
    sb2 = mod_b[:, D:2 * D]
    cb2 = mod_b[:, 2 * D:3 * D]
    gb = mod_b[:, 3 * D:4 * D]
    x1 = xf + ga * attn
    h2 = (_layernorm(x1) * (1.0 + cb2) + sb2).astype(BF16)

    y = None
    for i in range(NF):
        cp_g(i).wait()
        g = _mm(h2, wg_v[i])
        cp_u(i).wait()
        u = _mm(h2, wu_v[i])
        a = (_gelu_tanh(g) * u).astype(BF16)
        cp_d(i).wait()
        part = _mm(a, wd_v[i])
        y = part if y is None else y + part

    out = x1 + gb * y
    o_ref[...] = out[0:1, :].astype(o_ref.dtype)


@jax.jit
def pallas_adaLN_cond__sliding_block_cached__geglu_ffn__decode_kernel(
    A_x: jax.Array,
    A_k_cache: jax.Array,
    A_v_cache: jax.Array,
    A_wq: jax.Array,
    A_wo: jax.Array,
    B_x: jax.Array,
    B_w_gate: jax.Array,
    B_w_up: jax.Array,
    B_w_down: jax.Array,
    c: jax.Array,
    w_mod: jax.Array,
):
    del B_x
    B, Sq, D = A_x.shape
    _, H, S, DH = A_k_cache.shape
    W = min(4096, max(256, S // 4))
    F = B_w_gate.shape[1]
    assert B == 1 and Sq == 1 and H % 2 == 0 and F % FC == 0

    kT = jnp.transpose(A_k_cache[0], (0, 2, 1))
    vT = jnp.transpose(A_v_cache[0], (0, 2, 1))
    x2 = A_x.reshape(1, D)

    NP, NF = H // 2, F // FC
    nsem = 4 + WQ_CHUNKS + 2 * NSLOT + NP + 3 * NF
    any_spec = pl.BlockSpec(memory_space=pl.ANY)
    out = pl.pallas_call(
        functools.partial(_kernel, H=H, DH=DH, S=S, W=W, D=D, F=F),
        out_shape=jax.ShapeDtypeStruct((1, D), A_x.dtype),
        in_specs=[any_spec] * 10,
        out_specs=pl.BlockSpec(memory_space=pltpu.VMEM),
        scratch_shapes=[
            pltpu.VMEM((1, D), BF16),
            pltpu.VMEM((1, D), BF16),
            pltpu.VMEM((D, 6 * D), BF16),
            pltpu.VMEM((D, H * DH), BF16),
            pltpu.VMEM((NP, 2 * DH, D), BF16),
            pltpu.VMEM((NF, D, FC), BF16),
            pltpu.VMEM((NF, D, FC), BF16),
            pltpu.VMEM((NF, FC, D), BF16),
            pltpu.VMEM((NSLOT, DH, W), BF16),
            pltpu.VMEM((NSLOT, DH, W), BF16),
            pltpu.VMEM((M, H * DH), BF16),
            pltpu.SemaphoreType.DMA((nsem,)),
        ],
        compiler_params=pltpu.CompilerParams(vmem_limit_bytes=100 * 1024 * 1024),
    )(x2, kT, vT, A_wq, A_wo, B_w_gate, B_w_up, B_w_down, c, w_mod)
    return out.reshape(B, Sq, D)
```

```python
import functools

import jax
import jax.numpy as jnp
import jax.experimental.pallas as pl
import jax.experimental.pallas.tpu as pltpu

F32 = jnp.float32
BF16 = jnp.bfloat16

M = 8
NSLOT = 4
AHEAD = 3
D_CHUNKS = (768, 512, 256)
Q0ROWS = 16
CW = 128
WBLK = 128
WMODE = 'blk'
NOBOUNDS = False
NOSEMCHK = False
GU_Q = -1
TAIL_Q = 1


def _layernorm(x, eps=1e-5):
    m = jnp.mean(x, axis=-1, keepdims=True)
    d = x - m
    v = jnp.mean(d * d, axis=-1, keepdims=True)
    return d * jax.lax.rsqrt(v + eps)


def _gelu_tanh(x):
    c0 = 0.7978845608028654
    return 0.5 * x * (1.0 + jnp.tanh(c0 * (x + 0.044715 * (x * x * x))))


def _mm(a, b):
    return jnp.dot(a, b, preferred_element_type=F32)


def _mm_nt(a, b):
    return jax.lax.dot_general(a, b, (((1,), (1,)), ((), ())), preferred_element_type=F32)


def _copy(src, dst, sem, queue):
    pltpu.make_async_copy(src, dst, sem).start(priority=queue)


def _start(src, dst, sem, queue=-1):
    nr, nc = src.shape
    if queue >= 0:
        _copy(src, dst, sem, queue)
        return
    if WMODE == 'half' and nr != 192:
        h = nr // 2
        _copy(src.at[pl.ds(0, h)], dst.at[pl.ds(0, h)], sem, 0)
        _copy(src.at[pl.ds(h, nr - h)], dst.at[pl.ds(h, nr - h)], sem, 1)
        return
    blk = nr if nr == 192 else WBLK
    for r in range(0, nr, blk):
        lo, hi = pl.ds(r, Q0ROWS), pl.ds(r + Q0ROWS, blk - Q0ROWS)
        for c in range(0, nc, CW):
            cs = pl.ds(c, CW)
            _copy(src.at[lo, cs], dst.at[lo, cs], sem, 0)
            _copy(src.at[hi, cs], dst.at[hi, cs], sem, 1)


def _wait(dst, sem):
    pltpu.make_async_copy(dst, dst, sem).wait()


def _kernel(x_hbm, kT_hbm, vT_hbm, wq_hbm, wo_hbm, wg_hbm, wu_hbm, wd_hbm, c_hbm, wm_hbm,
            o_ref,
            x_v, c_v, wm_v, wq_v, wo_v, wg_v, wu_v, wd_v, k_v, v_v, q_s, sems,
            *, H, DH, S, W, D, F):
    NP = H // 2
    ND = len(D_CHUNKS)
    D_OFF = [sum(D_CHUNKS[:i]) for i in range(ND)]
    win = pl.ds(S - W, W)
    sem_w = sems.at[2 * NSLOT]

    def start_k(h):
        s = h % NSLOT
        _start(kT_hbm.at[h, :, win], k_v.at[s], sems.at[s])

    def start_v(h, odd):
        s = h % NSLOT
        _start(vT_hbm.at[h, :, win], v_v.at[s], sems.at[NSLOT + s])
        if odd:
            _start(wo_hbm.at[h // 2], wo_v.at[h // 2], sems.at[NSLOT + s])

    def d_sem(i):
        return sems.at[(0, 1, NSLOT, NSLOT + 1)[i]]

    def d_rows(i):
        return pl.ds(D_OFF[i], D_CHUNKS[i])

    _start(wm_hbm, wm_v, sem_w)
    pltpu.make_async_copy(c_hbm, c_v, sem_w).start()
    pltpu.make_async_copy(x_hbm, x_v, sem_w).start()
    _start(wq_hbm, wq_v, sem_w)
    start_k(0)
    start_v(0, False)
    start_k(1)
    start_v(1, True)
    start_k(2)

    _wait(wm_v, sem_w)
    _wait(c_v, sem_w)
    _wait(x_v, sem_w)
    _wait(wq_v, sem_w)
    cf = c_v[...].astype(F32)
    sc8 = jnp.broadcast_to(cf * jax.nn.sigmoid(cf), (M, D)).astype(BF16)
    mod = _mm(sc8, wm_v[...])
    sa, ca, ga, sb, cb, gb = (mod[:, i * D:(i + 1) * D] for i in range(6))
    xf = x_v[...].astype(F32)
    hb = (_layernorm(xf) * (1.0 + ca) + sa).astype(BF16)
    q_s[...] = _mm(hb, wq_v[...]).astype(BF16)

    scale = DH ** -0.5

    def head(hh, qh, odd):
        s_ = hh % NSLOT
        _wait(k_v.at[s_], sems.at[s_])

        @pl.when(hh + 2 < H)
        def _():
            start_v(hh + 2, odd)

        sc_ = _mm(qh, k_v[s_]) * scale
        e = jnp.exp(sc_ - jnp.max(sc_, axis=-1, keepdims=True))
        l = jnp.sum(e, axis=-1, keepdims=True)
        _wait(v_v.at[s_], sems.at[NSLOT + s_])
        if odd:
            _wait(wo_v.at[hh // 2], sems.at[NSLOT + s_])

        @pl.when(hh + 3 < H)
        def _():
            start_k(hh + 3)

        if odd:
            @pl.when(hh + 3 == H)
            def _():
                _start(wg_hbm, wg_v, sem_w, GU_Q)
                _start(wu_hbm, wu_v, sem_w, GU_Q)
                for i in range(ND):
                    _start(wd_hbm.at[d_rows(i)], wd_v.at[d_rows(i)], d_sem(i), TAIL_Q)

        return _mm_nt(e.astype(BF16), v_v[s_]) / l

    def pair(j, acc):
        qp = q_s[:, pl.ds(pl.multiple_of(j * 2 * DH, 2 * DH), 2 * DH)]
        oa = head(2 * j, qp[:, 0:DH], False)
        ob = head(2 * j + 1, qp[:, DH:2 * DH], True)
        op = jnp.concatenate([oa, ob], axis=-1).astype(BF16)
        return acc + _mm(op, wo_v[j])

    attn = jax.lax.fori_loop(0, NP, pair, jnp.zeros((M, D), F32))

    x1 = xf + ga * attn
    h2 = (_layernorm(x1) * (1.0 + cb) + sb).astype(BF16)
    _wait(wg_v, sem_w)
    _wait(wu_v, sem_w)
    a = (_gelu_tanh(_mm(h2, wg_v[...])) * _mm(h2, wu_v[...])).astype(BF16)
    y = None
    for i in range(ND):
        _wait(wd_v.at[d_rows(i)], d_sem(i))
        part = _mm(a[:, D_OFF[i]:D_OFF[i] + D_CHUNKS[i]], wd_v[d_rows(i), :])
        y = part if y is None else y + part

    out = x1 + gb * y
    o_ref[...] = out[0:1, :].astype(o_ref.dtype)


@jax.jit
def pallas_adaLN_cond__sliding_block_cached__geglu_ffn__decode_kernel(
    A_x: jax.Array,
    A_k_cache: jax.Array,
    A_v_cache: jax.Array,
    A_wq: jax.Array,
    A_wo: jax.Array,
    B_x: jax.Array,
    B_w_gate: jax.Array,
    B_w_up: jax.Array,
    B_w_down: jax.Array,
    c: jax.Array,
    w_mod: jax.Array,
):
    del B_x
    B, Sq, D = A_x.shape
    _, H, S, DH = A_k_cache.shape
    W = min(4096, max(256, S // 4))
    F = B_w_gate.shape[1]
    assert B == 1 and Sq == 1 and H % NSLOT == 0 and NSLOT == 4 and AHEAD == 3
    assert F == sum(D_CHUNKS) and len(D_CHUNKS) <= 4

    kT = jnp.transpose(A_k_cache[0], (0, 2, 1))
    vT = jnp.transpose(A_v_cache[0], (0, 2, 1))
    x2 = A_x.reshape(1, D)
    NP = H // 2
    wo3 = A_wo.reshape(NP, 2 * DH, D)

    any_spec = pl.BlockSpec(memory_space=pl.ANY)
    out = pl.pallas_call(
        functools.partial(_kernel, H=H, DH=DH, S=S, W=W, D=D, F=F),
        out_shape=jax.ShapeDtypeStruct((1, D), A_x.dtype),
        in_specs=[any_spec] * 10,
        out_specs=pl.BlockSpec(memory_space=pltpu.VMEM),
        scratch_shapes=[
            pltpu.VMEM((1, D), BF16),
            pltpu.VMEM((1, D), BF16),
            pltpu.VMEM((D, 6 * D), BF16),
            pltpu.VMEM((D, H * DH), BF16),
            pltpu.VMEM((NP, 2 * DH, D), BF16),
            pltpu.VMEM((D, F), BF16),
            pltpu.VMEM((D, F), BF16),
            pltpu.VMEM((F, D), BF16),
            pltpu.VMEM((NSLOT, DH, W), BF16),
            pltpu.VMEM((NSLOT, DH, W), BF16),
            pltpu.VMEM((M, H * DH), BF16),
            pltpu.SemaphoreType.DMA((2 * NSLOT + 1,)),
        ],
        compiler_params=pltpu.CompilerParams(disable_semaphore_checks=NOSEMCHK, disable_bounds_checks=NOBOUNDS, vmem_limit_bytes=100 * 1024 * 1024),
    )(x2, kT, vT, A_wq, wo3, B_w_gate, B_w_up, B_w_down, c, w_mod)
    return out.reshape(B, Sq, D)
```

```python
import functools

import jax
import jax.numpy as jnp
import jax.experimental.pallas as pl
import jax.experimental.pallas.tpu as pltpu

F32 = jnp.float32
BF16 = jnp.bfloat16

M = 8
NSLOT = 2
TR, TC = 8, 128
KV_Q0 = 16
GRP_MOD = (10, 2)
GRP_Q = (10, 1)
GRP_O = (12, 1)
GRP_GU = (10, 1)
D_CHUNKS = (768, 512, 256)


def _layernorm(x, eps=1e-5):
    m = jnp.mean(x, axis=-1, keepdims=True)
    d = x - m
    v = jnp.mean(d * d, axis=-1, keepdims=True)
    return d * jax.lax.rsqrt(v + eps)


def _gelu_tanh(x):
    c0 = 0.7978845608028654
    return 0.5 * x * (1.0 + jnp.tanh(c0 * (x + 0.044715 * (x * x * x))))


def _mm(a, b):
    return jnp.dot(a, b, preferred_element_type=F32)


def _mm_nt(a, b):
    return jax.lax.dot_general(a, b, (((1,), (1,)), ((), ())), preferred_element_type=F32)


def _copy(src, dst, sem, queue=0):
    pltpu.make_async_copy(src, dst, sem).start(priority=queue)


def _wait(dst, sem):
    pltpu.make_async_copy(dst, dst, sem).wait()


def _start_window(src, dst, sem):
    nr, nc = src.shape
    lo, hi = pl.ds(0, KV_Q0), pl.ds(KV_Q0, nr - KV_Q0)
    for c in range(0, nc, TC):
        cs = pl.ds(c, TC)
        _copy(src.at[lo, cs], dst.at[lo, cs], sem, 0)
        _copy(src.at[hi, cs], dst.at[hi, cs], sem, 1)


def _start_groups(src, dst, sem, g0, row0=0, nrows=None):
    g, r, nc = src.shape
    nrows = r if nrows is None else nrows
    lo, hi = pl.ds(0, g0), pl.ds(g0, g - g0)
    for a in range(0, nrows, TR):
        rs = pl.ds(row0 + a, TR)
        for c in range(0, nc, TC):
            cs = pl.ds(c, TC)
            _copy(src.at[lo, rs, cs], dst.at[lo, rs, cs], sem, 0)
            _copy(src.at[hi, rs, cs], dst.at[hi, rs, cs], sem, 1)


def _matrix(ref):
    g, r, c = ref.shape
    return ref[...].reshape(g * r, c)


def _kernel(x_hbm, kT_hbm, vT_hbm, wq_hbm, wo_hbm, wg_hbm, wu_hbm, wd_hbm, c_hbm, wm_hbm,
            o_ref,
            x_v, c_v, wm_v, wq_v, wo_v, wgu_v, wd_v, k_v, v_v, q_s, o_s, sems,
            *, H, DH, S, W, D):
    ND = len(D_CHUNKS)
    D_OFF = [sum(D_CHUNKS[:i]) for i in range(ND)]
    win = pl.ds(S - W, W)

    sem_w = sems.at[2 * NSLOT]
    sem_o = sems.at[2 * NSLOT + 1]

    def start_k(h):
        s = h % NSLOT
        _start_window(kT_hbm.at[h, :, win], k_v.at[s], sems.at[s])

    def start_v(h):
        s = h % NSLOT
        _start_window(vT_hbm.at[h, :, win], v_v.at[s], sems.at[NSLOT + s])

    def start_wo(h):
        n = wo_hbm.shape[1] // H
        _start_groups(wo_hbm, wo_v, sem_o, GRP_O[1], pl.multiple_of(h * n, n), n)

    def d_rows(i):
        return pl.ds(D_OFF[i], D_CHUNKS[i])

    def d_sem(i):
        return sems.at[(0, 1, NSLOT + (H - 2) % NSLOT)[i]]

    def start_ffn():
        _start_groups(wg_hbm, wgu_v.at[0], sem_w, GRP_GU[1])
        _start_groups(wu_hbm, wgu_v.at[1], sem_w, GRP_GU[1])
        for i in range(ND):
            _copy(wd_hbm.at[d_rows(i)], wd_v.at[d_rows(i)], d_sem(i), 1)

    _start_groups(wm_hbm, wm_v, sem_o, GRP_MOD[1])
    _copy(c_hbm, c_v, sems.at[0])
    _copy(x_hbm, x_v, sems.at[1])
    _start_groups(wq_hbm, wq_v, sem_w, GRP_Q[1])
    _wait(wm_v, sem_o)
    _wait(c_v, sems.at[0])
    _wait(x_v, sems.at[1])
    cf = c_v[...].astype(F32)
    silu_c = jnp.broadcast_to(cf * jax.nn.sigmoid(cf), (M, D)).astype(BF16)
    mod = _mm(silu_c, _matrix(wm_v))
    sa, ca, ga, sb, cb, gb = (mod[:, i * D:(i + 1) * D] for i in range(6))
    xf = x_v[...].astype(F32)
    h1 = (_layernorm(xf) * (1.0 + ca) + sa).astype(BF16)
    start_k(0)
    start_v(0)
    _wait(wq_v, sem_w)
    q_s[...] = _mm(h1, _matrix(wq_v)).astype(BF16)

    scale = DH ** -0.5

    def when_more(hh, odd, fn):
        if odd:
            pl.when(hh + 1 < H)(fn)
        else:
            fn()

    def head(hh, qh, odd):
        s_ = hh % NSLOT
        _wait(k_v.at[s_], sems.at[s_])
        when_more(hh, odd, lambda: start_k(hh + 1))
        start_wo(hh)
        if odd:
            pl.when(hh + 1 == H)(start_ffn)

        scores = _mm(qh, k_v[s_]) * scale
        e = jnp.exp(scores - jnp.max(scores, axis=-1, keepdims=True))
        denom = jnp.sum(e, axis=-1, keepdims=True)
        _wait(v_v.at[s_], sems.at[NSLOT + s_])
        when_more(hh, odd, lambda: start_v(hh + 1))
        return _mm_nt(e.astype(BF16), v_v[s_]) / denom

    def pair(j, carry):
        cols = pl.ds(pl.multiple_of(j * 2 * DH, 2 * DH), 2 * DH)
        qp = q_s[:, cols]
        oa = head(2 * j, qp[:, 0:DH], False)
        ob = head(2 * j + 1, qp[:, DH:2 * DH], True)
        o_s[:, cols] = jnp.concatenate([oa, ob], axis=-1).astype(BF16)
        return carry

    jax.lax.fori_loop(0, H // 2, pair, 0)

    _wait(wo_v, sem_o)
    x1 = xf + ga * _mm(o_s[...], _matrix(wo_v))
    h2 = (_layernorm(x1) * (1.0 + cb) + sb).astype(BF16)
    _wait(wgu_v, sem_w)
    gate = _mm(h2, _matrix(wgu_v.at[0]))
    up = _mm(h2, _matrix(wgu_v.at[1]))
    act = (_gelu_tanh(gate) * up).astype(BF16)
    y = None
    for i in range(ND):
        _wait(wd_v.at[d_rows(i)], d_sem(i))
        part = _mm(act[:, D_OFF[i]:D_OFF[i] + D_CHUNKS[i]], wd_v[d_rows(i), :])
        y = part if y is None else y + part

    out = x1 + gb * y
    o_ref[...] = out[0:1, :].astype(o_ref.dtype)


@jax.jit
def pallas_adaLN_cond__sliding_block_cached__geglu_ffn__decode_kernel(
    A_x: jax.Array,
    A_k_cache: jax.Array,
    A_v_cache: jax.Array,
    A_wq: jax.Array,
    A_wo: jax.Array,
    B_x: jax.Array,
    B_w_gate: jax.Array,
    B_w_up: jax.Array,
    B_w_down: jax.Array,
    c: jax.Array,
    w_mod: jax.Array,
):
    del B_x
    B, Sq, D = A_x.shape
    _, H, S, DH = A_k_cache.shape
    W = min(4096, max(256, S // 4))
    F = B_w_gate.shape[1]
    assert (B, Sq, D, H, DH, F) == (1, 1, 640, 32, 192, 1536) and A_wq.shape == (D, H * DH)
    assert W % TC == 0 and (S - W) % TC == 0 and F == sum(D_CHUNKS) and len(D_CHUNKS) <= 3

    kT = jnp.transpose(A_k_cache[0], (0, 2, 1))
    vT = jnp.transpose(A_v_cache[0], (0, 2, 1))
    x2 = A_x.reshape(1, D)

    def grouped(a, grp):
        return a.reshape(grp[0], a.shape[0] // grp[0], a.shape[1])

    wm3, wq3, wo3 = grouped(w_mod, GRP_MOD), grouped(A_wq, GRP_Q), grouped(A_wo, GRP_O)
    wg3, wu3 = grouped(B_w_gate, GRP_GU), grouped(B_w_up, GRP_GU)

    def like(a):
        return pltpu.VMEM(a.shape, BF16)

    out = pl.pallas_call(
        functools.partial(_kernel, H=H, DH=DH, S=S, W=W, D=D),
        out_shape=jax.ShapeDtypeStruct((1, D), A_x.dtype),
        in_specs=[pl.BlockSpec(memory_space=pl.ANY)] * 10,
        out_specs=pl.BlockSpec(memory_space=pltpu.VMEM),
        scratch_shapes=[
            like(x2), like(c), like(wm3), like(wq3), like(wo3),
            pltpu.VMEM((2,) + wg3.shape, BF16),
            like(B_w_down),
            pltpu.VMEM((NSLOT, DH, W), BF16),
            pltpu.VMEM((NSLOT, DH, W), BF16),
            pltpu.VMEM((M, H * DH), BF16),
            pltpu.VMEM((M, H * DH), BF16),
            pltpu.SemaphoreType.DMA((2 * NSLOT + 2,)),
        ],
        compiler_params=pltpu.CompilerParams(vmem_limit_bytes=64 * 1024 * 1024),
    )(x2, kT, vT, wq3, wo3, wg3, wu3, B_w_down, c, wm3)
    return out.reshape(B, Sq, D)
```
